```python
import os as _os
_os.environ.setdefault('JAX_PLATFORMS', 'cpu')
import jax
import jax.numpy as jnp

def _softmax(x, axis=-1):
    return jax.nn.softmax(x, axis=axis)

def _gelu(x):
    return jax.nn.gelu(x, approximate=True)

def _silu(x):
    return jax.nn.silu(x)

def _sigmoid(x):
    return jax.nn.sigmoid(x)

def _layernorm(x, axis=-1, eps=1e-05):
    m = jnp.mean(x, axis=axis, keepdims=True)
    v = jnp.var(x, axis=axis, keepdims=True)
    return (x - m) / jnp.sqrt(v + eps)

def _scatter_add(tgt, idx, src, axis=0):
    return tgt.at[idx].add(src)

def _segment_sum(src, seg, n):
    return jax.ops.segment_sum(src, seg, n)

class _Rng:

    def __init__(self, key):
        self._k = key

    def _next(self):
        self._k, sub = jax.random.split(self._k)
        return sub

    def normal(self, shape):
        return jax.random.normal(self._next(), shape, dtype=jnp.bfloat16)

    def randint(self, lo, hi, shape):
        return jax.random.randint(self._next(), shape, lo, hi, dtype=jnp.int32)

    def uniform(self, shape, lo=0.0, hi=1.0):
        return jax.random.uniform(self._next(), shape, jnp.bfloat16, lo, hi)

    def permutation(self, n):
        return jax.random.permutation(self._next(), n)
kernel_name = 'gated_mix__memory_aug_recurrent_mem_tr__glu_gated_geglu__prompt'

def setup_inputs():
    _rng = _Rng(jax.random.key(int.from_bytes(__import__("os").urandom(4), "little")))
    _w = lambda a: (lambda t: t.astype(jnp.bfloat16) if jnp.issubdtype(t.dtype, jnp.floating) else t)(jnp.asarray(a))

    def _A_setup():
        B, S, Dm = (1, 2048, 640)
        H, Dh = (32, 128)
        M, seg = (8, 32)
        seg = min(seg, S)
        S = S // seg * seg
        return {'x': _w((lambda *s: _rng.normal(s) * 0.05)(B, S, Dm)), 'mem0': _w((lambda *s: _rng.normal(s) * 0.4)(B, M, Dm)), 'Wq': _w((lambda *s: _rng.normal(s) * 3.2)(Dm, H, Dh) * Dm ** (-0.5)), 'Wk': _w((lambda *s: _rng.normal(s) * 3.2)(Dm, H, Dh) * Dm ** (-0.5)), 'Wv': _w((lambda *s: _rng.normal(s) * 0.4)(Dm, H, Dh) * Dm ** (-0.5)), 'Wo': _w((lambda *s: _rng.normal(s) * 0.4)(H, Dh, Dm) * (H * Dh) ** (-0.5)), 'seg_len': seg}
    _A_in = _A_setup()

    def _B_setup():
        B, S, Dm, Df = (1, 2048, 640, 1728)
        return {'x': _w((lambda *s: _rng.normal(s) * 0.05)(B, S, Dm)), 'w_gate': _w((lambda *s: _rng.normal(s) * 1.6)(Dm, Df) * Dm ** (-0.5)), 'w_up': _w((lambda *s: _rng.normal(s) * 1.6)(Dm, Df) * Dm ** (-0.5)), 'w_down': _w((lambda *s: _rng.normal(s) * 1.6)(Df, Dm) * Df ** (-0.5))}
    _B_in = _B_setup()
    return {'A_x': _A_in['x'], 'A_mem0': _A_in['mem0'], 'A_Wq': _A_in['Wq'], 'A_Wk': _A_in['Wk'], 'A_Wv': _A_in['Wv'], 'A_Wo': _A_in['Wo'], 'A_seg_len': _A_in['seg_len'], 'B_x': _B_in['x'], 'B_w_gate': _B_in['w_gate'], 'B_w_up': _B_in['w_up'], 'B_w_down': _B_in['w_down'], 'gate_w': _w((lambda *s: _rng.normal(s) * 0.05)(640) * 16.0)}

def reference(A_x, A_mem0, A_Wq, A_Wk, A_Wv, A_Wo, A_seg_len, B_x, B_w_gate, B_w_up, B_w_down, gate_w):

    def _A_ref(x, mem0, Wq, Wk, Wv, Wo, seg_len):
        B, S, Dm = x.shape
        H, Dh = (Wq.shape[1], Wq.shape[2])
        M = mem0.shape[1]
        scale = Dh ** (-0.5)
        n_seg = S // seg_len
        L = M + seg_len
        idx = jnp.arange(L)
        mask = (idx[:, None] < M) | (idx[:, None] >= idx[None, :])
        mem = mem0
        outs = []
        for s in range(n_seg):
            xs = x[:, s * seg_len:(s + 1) * seg_len, :].copy()
            h = jnp.concatenate([mem, xs], axis=1)
            q = jnp.einsum('btd,dhe->bhte', h, Wq)
            k = jnp.einsum('btd,dhe->bhte', h, Wk)
            v = jnp.einsum('btd,dhe->bhte', h, Wv)
            scores = jnp.einsum('bhqe,bhke->bhqk', q, k) * scale
            scores = jnp.where(mask[None, None], scores, -1000000000.0)
            p = _softmax(scores, axis=-1)
            o = jnp.einsum('bhqk,bhke->bhqe', p, v)
            o = jnp.einsum('bhte,hed->btd', o, Wo)
            mem = o[:, :M, :].copy()
            outs.append(o[:, M:, :])
        return jnp.concatenate(outs, axis=1)

    def _B_ref(x, w_gate, w_up, w_down):
        g = jnp.einsum('bsd,df->bsf', x, w_gate)
        u = jnp.einsum('bsd,df->bsf', x, w_up)
        h = _gelu(g) * u
        return jnp.einsum('bsf,fd->bsd', h, w_down)
    x = A_x
    g = _sigmoid((x * gate_w).sum(-1, keepdims=True))
    a = _A_ref(x, A_mem0, A_Wq, A_Wk, A_Wv, A_Wo, A_seg_len)
    b = _B_ref(x, B_w_gate, B_w_up, B_w_down)
    return g * a + (1 - g) * b
```

```python
import functools

import jax
import jax.numpy as jnp
import jax.experimental.pallas as pl
import jax.experimental.pallas.tpu as pltpu

F32 = jnp.float32
BF16 = jnp.bfloat16
LOG2E = 1.4426950408889634


def _group_mask(nh, seg, nm, rows):
    r = jax.lax.broadcasted_iota(jnp.int32, (rows, rows), 0)
    c = jax.lax.broadcasted_iota(jnp.int32, (rows, rows), 1)
    nx = nh * seg

    def head_pos(i):
        is_x = i < nx
        head = jnp.where(is_x, i // seg, (i - nx) // nm)
        pos = i % seg
        return is_x, head, pos

    r_x, r_h, r_p = head_pos(r)
    c_x, c_h, c_p = head_pos(c)
    real = (r < nx + nh * nm) & (c < nx + nh * nm)
    vis = jnp.logical_not(r_x) | jnp.logical_not(c_x) | (r_p >= c_p)
    return real & (r_h == c_h) & vis


def _kernel(x_hbm, mem_hbm, wq_hbm, wk_hbm, wv_hbm, wo_hbm, wg_hbm, wu_hbm, wd_hbm, gw_hbm,
            out_hbm,
            x_v, mem0_v, gw_v, stage, wqkv, wo_v, wg_v, wu_v, wd_v,
            acc, gate_v, out_v, h_v, mem_v, stash_qkv, stash_o, o_v, bias_v, sems,
            *, S, D, H, E, NM, SEG, DF):
    scale = E ** (-0.5)
    HP = H // 2

    RB0 = 256
    RB = 128
    FC = 256
    NWC = 12
    DC = 3 * D // NWC
    DB = 32
    X0 = RB0 + RB
    fchunks = [(c0, min(FC, DF - c0)) for c0 in range(0, DF, FC)]
    KH = 896

    def cp(src, dst, k):
        return pltpu.make_async_copy(src, dst, sems.at[k])

    sem_id = [0]

    def new_cp(src, dst):
        c = cp(src, dst, sem_id[0])
        sem_id[0] += 1
        return c

    cp_x0 = new_cp(x_hbm.at[pl.ds(0, X0)], x_v.at[pl.ds(0, X0)])
    cp_gw = new_cp(gw_hbm, gw_v)
    cp_g = [new_cp(wg_hbm.at[pl.ds(c0, cw)], wg_v.at[pl.ds(c0, cw)]) for c0, cw in fchunks]
    cp_u = [new_cp(wu_hbm.at[pl.ds(c0, cw)], wu_v.at[pl.ds(c0, cw)]) for c0, cw in fchunks]
    cp_d = [new_cp(wd_hbm.at[pl.ds(0, KH)], wd_v.at[pl.ds(0, KH)]),
            new_cp(wd_hbm.at[pl.ds(KH, DF - KH)], wd_v.at[pl.ds(KH, DF - KH)])]
    cp_x1 = new_cp(x_hbm.at[pl.ds(X0, S - X0)], x_v.at[pl.ds(X0, S - X0)])
    cp_mem = new_cp(mem_hbm, mem0_v)
    cp_wo = new_cp(wo_hbm, wo_v)
    W_SEM0 = sem_id[0]
    w_hbms = (wq_hbm, wk_hbm, wv_hbm)
    per_mat = NWC // 3
    cp_w = [new_cp(w_hbms[k // per_mat].at[pl.ds((k % per_mat) * DC * H, DC * H)],
                   stage.at[pl.ds(k * DC * H, DC * H)]) for k in range(NWC)]
    OUT_SEM0 = sem_id[0]

    cp_x0.start()
    cp_gw.start()
    for a, b in zip(cp_g, cp_u):
        a.start()
        b.start()
    cp_d[0].start()
    cp_d[1].start()
    cp_w[0].start()
    cp_x1.start()
    for c in cp_w[1:]:
        c.start()
    cp_wo.start()
    cp_mem.start()

    bias_v[0] = jnp.where(_group_mask(3, SEG, NM, 128), 0.0, -1e9).astype(F32)
    bias_v[1] = jnp.where(_group_mask(2, SEG, NM, 128), 0.0, -1e9).astype(F32)

    NT = (((1,), (1,)), ((), ()))
    su = stage.bitcast(jnp.uint32)

    def ffn_block(r0, rb, first, side=()):
        side = list(side)
        n_slots = 2 * len(fchunks) + D // 128 - 3
        per = -(-len(side) // n_slots)

        prev = []

        def run_side(cur):
            todo = per
            if side and prev:
                pv_ = prev[-1]
                pts = [(r, c) for c in range(0, pv_.shape[1] - 127, 128) for r in range(0, rb, 32)]
                pts = pts[::max(1, len(pts) // per)][:per]
                for (r, c) in pts:
                    if side and todo:
                        su[3 * D * HP:3 * D * HP + 8, :] = pltpu.bitcast(pv_[r:r + 8, c:c + 128], jnp.uint32)
                        side.pop(0)()
                        todo -= 1
            prev.append(cur)
            for _ in range(todo):
                if side:
                    side.pop(0)()

        xb = x_v[pl.ds(r0, rb), :]
        gw = gw_v[...].astype(F32).reshape(1, D)
        z = jnp.sum(xb.astype(F32) * gw, axis=-1, keepdims=True)
        gt = jax.nn.sigmoid(z)
        gate_v[pl.ds(r0, rb), :] = jnp.broadcast_to(gt, (rb, 128))
        for ci, (c0, cw) in enumerate(fchunks):
            if first:
                cp_g[ci].wait()
                cp_u[ci].wait()
            g = jax.lax.dot_general(xb, wg_v[c0:c0 + cw, :], NT, preferred_element_type=F32)
            run_side(g)
            u = jax.lax.dot_general(xb, wu_v[c0:c0 + cw, :], NT, preferred_element_type=F32)
            run_side(u)
            h_v[0:rb, c0:c0 + cw] = (jax.nn.gelu(g, approximate=True) * u).astype(BF16)
        if first:
            cp_d[0].wait()
            b = jnp.dot(h_v[0:rb, 0:KH], wd_v[0:KH, :], preferred_element_type=F32)
            cp_d[1].wait()
            b = b + jnp.dot(h_v[0:rb, KH:DF], wd_v[KH:DF, :], preferred_element_type=F32)
            acc[pl.ds(r0, rb), :] = (1.0 - gt) * b
        else:
            for n0 in range(0, D, 128):
                b = jnp.dot(h_v[0:rb, :], wd_v[:, n0:n0 + 128], preferred_element_type=F32)
                run_side(b)
                acc[pl.ds(r0, rb), n0:n0 + 128] = (1.0 - gt) * b
        while side:
            side.pop(0)()

    cp_x0.wait()
    cp_gw.wait()
    ffn_block(0, RB0, True)

    def relayout_chunk(k):
        m = k // per_mat
        dbase = (k % per_mat) * DC
        thunks = []
        for ub in range(DC // DB):
            d0 = pl.multiple_of(dbase + ub * DB, DB)
            blk = su.at[pl.ds(pl.multiple_of((k * DC + ub * DB) * HP, DB * HP), DB * HP)]
            for j in range(HP):
                def piece(d0=d0, blk=blk, j=j):
                    w = blk[pl.ds(j, DB, stride=HP), :]
                    lo = pltpu.bitcast(w << 16, F32).astype(BF16)
                    hi = pltpu.bitcast(w & jnp.uint32(0xFFFF0000), F32).astype(BF16)
                    wqkv[m * H + 2 * j, pl.ds(d0, DB), :] = lo
                    wqkv[m * H + 2 * j + 1, pl.ds(d0, DB), :] = hi
                thunks.append(piece)
        return thunks

    def ffn_loop(i, carry):
        @pl.when(i == 1)
        def _():
            cp_x1.wait()

        @pl.when(i < NWC)
        def _():
            dst = stage.at[pl.ds(pl.multiple_of(i * (DC * H), DC * H), DC * H)]
            pltpu.make_async_copy(dst, dst, sems.at[W_SEM0 + i]).wait()

        side = relayout_chunk(jnp.minimum(i, NWC - 1))
        ffn_block(pl.multiple_of(RB0 + i * RB, RB), RB, False, side)
        return carry

    jax.lax.fori_loop(0, (S - RB0) // RB, ffn_loop, 0)

    cp_wo.wait()
    cp_mem.wait()
    mem_v[...] = mem0_v[...].astype(F32)

    groups = []
    h0 = 0
    while h0 < H:
        n = min(3, H - h0)
        groups.append((h0, n))
        h0 += n

    zeros8 = jnp.zeros((8, E), F32)
    NG = len(groups)
    c_exp = scale * LOG2E

    def sub_step(h, even, pv_delay):
        M = h.shape[0]
        stk = {}
        sc = {}
        pr = {}

        def proj(t, g):
            g0, n = groups[g]
            px, pm = [], []
            for i in range(n):
                hh = g0 + i
                y = jnp.dot(h, wqkv[t * H + hh], preferred_element_type=F32)
                if even:
                    px.append(y[0:32])
                    stash_qkv[t * H + hh] = y[32:40]
                    pm.append(y[40:48])
                else:
                    px.append(jnp.concatenate([stash_qkv[t * H + hh], y[8:32]], axis=0))
                    pm.append(y[0:8])
            pad = 128 - n * (SEG + NM)
            stk[(t, g)] = jnp.concatenate(px + pm + [zeros8] * (pad // 8), axis=0).astype(BF16)

        def scores(g):
            n = groups[g][1]
            s = jax.lax.dot_general(stk.pop((0, g)), stk.pop((1, g)), (((1,), (1,)), ((), ())),
                                    preferred_element_type=F32)
            s = s + bias_v[0 if n == 3 else 1]
            m = jnp.max(s, axis=-1, keepdims=True)
            p = jnp.exp2((s - m) * c_exp)
            l = jnp.sum(p, axis=-1, keepdims=True)
            pr[g] = (p.astype(BF16), l)

        def pv(g):
            g0, n = groups[g]
            p, l = pr.pop(g)
            o3 = jnp.dot(p, stk.pop((2, g)), preferred_element_type=F32)
            r = pl.reciprocal(l, approx=True)
            r = r * (2.0 - l * r)
            o3 = o3 * r
            for i in range(n):
                hh = g0 + i
                ox = o3[i * SEG:(i + 1) * SEG]
                om = o3[n * SEG + i * NM:n * SEG + (i + 1) * NM]
                if even:
                    o_v[0:32, hh * E:(hh + 1) * E] = jnp.concatenate(
                        [ox[0:24], om], axis=0).astype(BF16)
                    stash_o[hh] = ox[24:32]
                else:
                    o_v[:, hh * E:(hh + 1) * E] = jnp.concatenate(
                        [stash_o[hh], om, ox], axis=0).astype(BF16)

        MO = 32 if even else 48

        def oproj(ga, gb):
            k0 = groups[ga][0] * E
            k1 = (groups[gb - 1][0] + groups[gb - 1][1]) * E
            return jnp.dot(o_v[0:MO, k0:k1], wo_v[k0:k1, :], preferred_element_type=F32)

        for g in range(NG):
            proj(1, g)
            if g - pv_delay >= 0:
                pv(g - pv_delay)
            proj(0, g)
            proj(2, g)
            scores(g)
        rest = list(range(NG - pv_delay, NG))
        res = oproj(0, 3)
        for idx, g in enumerate(rest[:-1]):
            pv(g)
        res = res + oproj(3, 7)
        pv(rest[-1])
        res = res + oproj(7, NG - 1)
        res = res + oproj(NG - 1, NG)
        return res

    def super_step(j, carry):
        r0 = pl.multiple_of(j * 64, 64)
        xa = x_v[pl.ds(r0, 32), :]
        xmid = x_v[pl.ds(r0 + 32, 16), :].astype(F32)
        xb = x_v[pl.ds(r0 + 48, 16), :]

        h_e = jnp.concatenate(
            [xa, jnp.concatenate([xmid[:8], mem_v[...]], axis=0).astype(BF16)], axis=0)
        res = sub_step(h_e, True, 2)
        gt = gate_v[pl.ds(r0, 24), :]
        acc[pl.ds(r0, 24), :] = acc[pl.ds(r0, 24), :] + jnp.concatenate([gt] * (D // 128), axis=1) * res[0:24]
        mem1 = res[24:32]

        h_o = jnp.concatenate(
            [jnp.concatenate([mem1, xmid[8:]], axis=0).astype(BF16), xb], axis=0)
        res = sub_step(h_o, False, 2)
        a = jnp.concatenate([res[0:8], res[16:48]], axis=0)
        gt = gate_v[pl.ds(r0 + 24, 40), :]
        acc[pl.ds(r0 + 24, 40), :] = acc[pl.ds(r0 + 24, 40), :] + jnp.concatenate([gt] * (D // 128), axis=1) * a
        mem_v[...] = res[8:16]
        out_v[pl.ds(r0, 64), :] = acc[pl.ds(r0, 64), :].astype(BF16)
        pltpu.make_async_copy(out_v.at[pl.ds(r0, 64)], out_hbm.at[pl.ds(r0, 64)],
                              sems.at[OUT_SEM0]).start()
        return carry

    jax.lax.fori_loop(0, S // 64, super_step, 0)

    pltpu.make_async_copy(out_v, out_hbm, sems.at[OUT_SEM0]).wait()


@functools.partial(jax.jit, static_argnames=("A_seg_len",))
def pallas_gated_mix__memory_aug_recurrent_mem_tr__glu_gated_geglu__prompt_kernel(
    A_x, A_mem0, A_Wq, A_Wk, A_Wv, A_Wo, A_seg_len, B_x, B_w_gate, B_w_up, B_w_down, gate_w,
):
    B, S, D = A_x.shape
    _, H, E = A_Wq.shape
    NM = A_mem0.shape[1]
    DF = B_w_gate.shape[1]
    SEG = int(A_seg_len)
    assert B == 1 and SEG == 32 and NM == 8 and E == 128 and S % 64 == 0 and H % 2 == 0

    kernel = functools.partial(_kernel, S=S, D=D, H=H, E=E, NM=NM, SEG=SEG, DF=DF)
    any_spec = pl.BlockSpec(memory_space=pltpu.HBM)
    out = pl.pallas_call(
        kernel,
        out_shape=jax.ShapeDtypeStruct((S, D), BF16),
        in_specs=[any_spec] * 10,
        out_specs=any_spec,
        scratch_shapes=[
            pltpu.VMEM((S, D), BF16),
            pltpu.VMEM((NM, D), BF16),
            pltpu.VMEM((D,), BF16),
            pltpu.VMEM((3 * D * H + 16, E), BF16),
            pltpu.VMEM((3 * H, D, E), BF16),
            pltpu.VMEM((H * E, D), BF16),
            pltpu.VMEM((DF, D), BF16),
            pltpu.VMEM((DF, D), BF16),
            pltpu.VMEM((DF, D), BF16),
            pltpu.VMEM((S, D), F32),
            pltpu.VMEM((S, 128), F32),
            pltpu.VMEM((S, D), BF16),
            pltpu.VMEM((256, DF), BF16),
            pltpu.VMEM((NM, D), F32),
            pltpu.VMEM((3 * H, 8, E), F32),
            pltpu.VMEM((H, 8, E), F32),
            pltpu.VMEM((48, H * E), BF16),
            pltpu.VMEM((2, 128, 128), F32),
            pltpu.SemaphoreType.DMA((48,)),
        ],
        compiler_params=pltpu.CompilerParams(vmem_limit_bytes=110 * 1024 * 1024),
    )(
        A_x.reshape(S, D), A_mem0.reshape(NM, D),
        A_Wq.reshape(D * H, E), A_Wk.reshape(D * H, E), A_Wv.reshape(D * H, E),
        A_Wo.reshape(H * E, D), B_w_gate.T, B_w_up.T, B_w_down, gate_w,
    )
    return out.reshape(B, S, D)
```

```python
import functools

import jax
import jax.numpy as jnp
import jax.experimental.pallas as pl
import jax.experimental.pallas.tpu as pltpu

F32 = jnp.float32
BF16 = jnp.bfloat16
LOG2E = 1.4426950408889634
NT = (((1,), (1,)), ((), ()))

RB0 = 256
RB = 256
FC = 256
DB = 32
FR = 64
WP = 324
PIECE = 2
UNROLL = 2


def _group_mask(nh, seg, nm, rows):
    r = jax.lax.broadcasted_iota(jnp.int32, (rows, rows), 0)
    c = jax.lax.broadcasted_iota(jnp.int32, (rows, rows), 1)
    nx = nh * seg

    def head_pos(i):
        is_x = i < nx
        head = jnp.where(is_x, i // seg, (i - nx) // nm)
        pos = i % seg
        return is_x, head, pos

    r_x, r_h, r_p = head_pos(r)
    c_x, c_h, c_p = head_pos(c)
    real = (r < nx + nh * nm) & (c < nx + nh * nm)
    vis = jnp.logical_not(r_x) | jnp.logical_not(c_x) | (r_p >= c_p)
    return real & (r_h == c_h) & vis


def _kernel(x_hbm, mem_hbm, wq_hbm, wk_hbm, wv_hbm, wo_hbm, wg_hbm, wu_hbm, wd_hbm, gw_hbm,
            out_hbm,
            x_v, mem0_v, gw_v, stage, wqkv, wo_v, wg_v, wu_v, wd_v, wt_v,
            acc_a, acc_b, gate_v, out_v, h_v, hf_v, mem_v, stash_qkv, stash_o, o_v, bias_v, sems,
            *, S, D, H, E, NM, SEG, DF):
    scale = E ** (-0.5)
    wqkv_u = wqkv.bitcast(jnp.uint32)
    wo_u = wo_v.bitcast(jnp.uint32)
    o_u = o_v.bitcast(jnp.uint32)
    HP = H // 2
    DFP = wg_v.shape[0]
    DFA = (DF // 128) * 128
    DFH = DFP // 2
    NBODY = S // (64 * UNROLL)
    F0 = S - FR * (NBODY // 2)
    X0 = RB0 + RB
    n_ffn = (F0 - RB0) // RB
    n_wg = n_ffn - 1
    DC = 3 * D // n_wg
    assert DC * n_wg == 3 * D and DC % DB == 0
    NU = 3 * D // DB
    fchunks = [(c0, min(FC, DFA - c0)) for c0 in range(0, DFA, FC)]
    KH = 896

    sem_id = [0]

    def new_cp(src, dst):
        c = pltpu.make_async_copy(src, dst, sems.at[sem_id[0]])
        sem_id[0] += 1
        return c

    def rows(ref, a, n):
        return ref.at[pl.ds(a, n)]

    TL = DF - DFA
    cp_x0 = new_cp(rows(x_hbm, 0, RB0), rows(x_v, 0, RB0))
    cp_x0b = new_cp(rows(x_hbm, RB0, X0 - RB0), rows(x_v, RB0, X0 - RB0))
    cp_gw = new_cp(gw_hbm, gw_v)
    cp_g = [new_cp(rows(wg_hbm, c0, cw), rows(wg_v, c0, cw)) for c0, cw in fchunks]
    cp_u = [new_cp(rows(wu_hbm, c0, cw), rows(wu_v, c0, cw)) for c0, cw in fchunks]
    cp_t = [new_cp(rows(wg_hbm, DFA, TL), rows(wt_v, 0, TL)),
            new_cp(rows(wu_hbm, DFA, TL), rows(wt_v, TL, TL))]
    cp_d = [new_cp(rows(wd_hbm, 0, KH), rows(wd_v, 0, KH)),
            new_cp(rows(wd_hbm, KH, DF - KH), rows(wd_v, KH, DF - KH))]
    cp_x1 = new_cp(rows(x_hbm, X0, S - X0), rows(x_v, X0, S - X0))
    cp_late = [new_cp(mem_hbm, mem0_v),
               *[new_cp(wo_hbm.at[:, pl.ds(n * 128, 128)], wo_v.at[n]) for n in range(D // 128)],
               new_cp(rows(wg_hbm, DFA, TL), rows(wg_v, DFA, TL)),
               new_cp(rows(wu_hbm, DFA, TL), rows(wu_v, DFA, TL))]
    W_SEM0 = sem_id[0]
    w_hbms = (wq_hbm, wk_hbm, wv_hbm)
    cp_w = []
    for k in range(n_wg):
        grp = []
        a = k * DC
        while a < (k + 1) * DC:
            b = min((k + 1) * DC, (a // D + 1) * D)
            grp.append(pltpu.make_async_copy(
                rows(w_hbms[a // D], (a % D) * H, (b - a) * H),
                rows(stage, a * H, (b - a) * H), sems.at[W_SEM0 + k]))
            a = b
        cp_w.append(grp)
    sem_id[0] += n_wg
    OUT_SEM = sem_id[0]
    assert OUT_SEM < sems.shape[0]

    cp_x0.start()
    cp_gw.start()
    for a, b in zip(cp_g, cp_u):
        a.start()
        b.start()
    for c in (*cp_t, *cp_d, cp_x0b, cp_x1, *[c for grp in cp_w for c in grp], *cp_late):
        c.start()

    bias_v[0] = jnp.where(_group_mask(3, SEG, NM, 128), 0.0, -1e9 / scale).astype(F32)
    bias_v[1] = jnp.where(_group_mask(2, SEG, NM, 128), 0.0, -1e9 / scale).astype(F32)
    zpad = jnp.zeros((DFP - DF, D), BF16)
    wg_v[DF:DFP, :] = zpad
    wu_v[DF:DFP, :] = zpad
    wd_v[DF:DFP, :] = zpad
    acc_b[F0:S, :] = jnp.zeros((S - F0, D), F32)

    su = stage.bitcast(jnp.uint32)
    su[NU * DB * HP:(NU + 1) * DB * HP, :] = jnp.zeros((DB * HP, E), jnp.uint32)

    def gate_of(xb):
        gw = gw_v[...].astype(F32).reshape(1, D)
        z = jnp.sum(xb.astype(F32) * gw, axis=-1, keepdims=True)
        return jnp.broadcast_to(jax.nn.sigmoid(z), (xb.shape[0], 128))

    def fence(t):
        su[(NU + 1) * DB * HP:(NU + 1) * DB * HP + 8, :] = pltpu.bitcast(t, jnp.uint32)

    def act(g, u, omg):
        w = g.shape[1]
        om = omg[:, 0:w] if w <= 128 else jnp.concatenate([omg] * (w // 128), axis=1)
        return (jax.nn.gelu(g, approximate=True) * u * om).astype(BF16)

    def ffn_block(r0, rb, first, side=()):
        side = list(side)
        n_slots = 2 * len(fchunks) + D // 128 - 3
        per = -(-len(side) // n_slots)
        prev = []

        def run_side(cur):
            todo = per
            if side and prev:
                pv_ = prev[-1]
                pts = [(r, c) for c in range(0, pv_.shape[1] - 127, 128) for r in range(0, rb, 32)]
                pts = pts[::max(1, len(pts) // per)][:per]
                for (r, c) in pts:
                    if side and todo:
                        fence(pv_[r:r + 8, c:c + 128])
                        side.pop(0)()
                        todo -= 1
            prev.append(cur)
            for _ in range(todo):
                if side:
                    side.pop(0)()

        xb = x_v[pl.ds(r0, rb), :]
        gt = gate_of(xb)
        gate_v[pl.ds(r0, rb), :] = gt
        omg = 1.0 - gt
        for ci, (c0, cw) in enumerate(fchunks):
            if first and ci < len(fchunks) - 1:
                cp_g[ci].wait()
                cp_u[ci].wait()
                if ci == len(fchunks) - 2:
                    for c in (cp_g[ci + 1], cp_u[ci + 1], *cp_t):
                        c.wait()
            g = jax.lax.dot_general(xb, wg_v[c0:c0 + cw, :], NT, preferred_element_type=F32)
            run_side(g)
            u = jax.lax.dot_general(xb, wu_v[c0:c0 + cw, :], NT, preferred_element_type=F32)
            run_side(u)
            h_v[0:rb, c0:c0 + cw] = act(g, u, omg)
        y = jax.lax.dot_general(xb, wt_v[...], NT, preferred_element_type=F32)
        h_v[0:rb, DFA:DF] = act(y[:, 0:TL], y[:, TL:2 * TL], omg)
        if first:
            cp_d[0].wait()
            b = jnp.dot(h_v[0:rb, 0:KH], wd_v[0:KH, :], preferred_element_type=F32)
            cp_d[1].wait()
            cp_x0b.wait()
            b = jnp.dot(h_v[0:rb, KH:DF], wd_v[KH:DF, :], preferred_element_type=F32) + b
            acc_b[pl.ds(r0, rb), :] = b
        else:
            for n0 in range(0, D, 128):
                b = jnp.dot(h_v[0:rb, :], wd_v[0:DF, n0:n0 + 128], preferred_element_type=F32)
                run_side(b)
                acc_b[pl.ds(r0, rb), n0:n0 + 128] = b
        while side:
            side.pop(0)()

    cp_x0.wait()
    cp_gw.wait()
    ffn_block(0, RB0, True)

    def relayout_chunk(k):
        thunks = []
        for ub in range(DC // DB):
            unit = jnp.where(k >= 0, k * (DC // DB) + ub, NU)
            m = unit // (D // DB)
            blk = su.at[pl.ds(pl.multiple_of(unit * (DB * HP), DB * HP), DB * HP)]
            base = m * (H * WP) + (unit % (D // DB)) * (DB // 2)
            dst = wqkv_u.at[pl.ds(pl.multiple_of(base, 8), (H - 1) * WP + DB // 2)]
            for dq in range(0, DB // 2, PIECE):
                def piece(blk=blk, dst=dst, dq=dq):
                    for dp in range(dq, dq + PIECE):
                        for jh in range(0, HP, 8):
                            a = blk[pl.ds(2 * dp * HP + jh, 8), :]
                            b = blk[pl.ds((2 * dp + 1) * HP + jh, 8), :]
                            dst[pl.ds(jh * WP + dp, 8, stride=WP), :] = (a & jnp.uint32(0xFFFF)) | (b << 16)
                            dst[pl.ds((HP + jh) * WP + dp, 8, stride=WP), :] = (
                                (a >> 16) | (b & jnp.uint32(0xFFFF0000)))
                thunks.append(piece)
        return thunks

    def ffn_loop(i, carry):
        @pl.when(i == 1)
        def _():
            cp_x1.wait()

        @pl.when(i >= 1)
        def _():
            dst = stage.at[pl.ds(pl.multiple_of((i - 1) * (DC * H), DC * H), DC * H)]
            pltpu.make_async_copy(dst, dst, sems.at[W_SEM0 + i - 1]).wait()

        r0 = pl.multiple_of(RB0 + i * RB, RB)
        ffn_block(r0, RB, False, relayout_chunk(i - 1))
        return carry

    jax.lax.fori_loop(0, n_ffn, ffn_loop, 0)

    for c in cp_late:
        c.wait()
    mem_v[...] = mem0_v[...].astype(F32)

    groups = []
    h0 = 0
    while h0 < H:
        n = min(3, H - h0)
        groups.append((h0, n))
        h0 += n
    zeros8 = jnp.zeros((8, E), F32)
    NG = len(groups)
    c_exp = scale * LOG2E

    def wtile(idx, k0, k1):
        m, hh = divmod(idx, H)
        r = (m * H + (hh % 2) * HP + hh // 2) * WP
        return pltpu.bitcast(wqkv_u[r + k0 // 2:r + k1 // 2, :], BF16)

    def sub_step(h, even, pv_delay, fill):
        stk = {}
        pr = {}

        def run_fill(key):
            for f in fill.get(key, ()):
                f()

        def nrows(n):
            return -(-(n * (SEG + NM)) // 16) * 16

        def proj(t, g, mid=None, mid_tile=0):
            g0, n = groups[g]
            px, pm = [], []
            kt = D // 128
            for i in range(n):
                hh = g0 + i
                ks = mid_tile - i * kt
                if mid is not None and 0 < ks < kt:
                    y = jnp.dot(h[:, :ks * 128], wtile(t * H + hh, 0, ks * 128),
                                preferred_element_type=F32)
                    mid()
                    y = jnp.dot(h[:, ks * 128:], wtile(t * H + hh, ks * 128, D),
                                preferred_element_type=F32) + y
                else:
                    if mid is not None and ks == 0:
                        mid()
                    y = jnp.dot(h, wtile(t * H + hh, 0, D), preferred_element_type=F32)
                if even:
                    px.append(y[0:32])
                    stash_qkv[t * H + hh] = y[32:40]
                    pm.append(y[40:48])
                else:
                    px.append(jnp.concatenate([stash_qkv[t * H + hh], y[8:32]], axis=0))
                    pm.append(y[0:8])
            pad = (nrows(n) if t == 0 else 128) - n * (SEG + NM)
            stk[(t, g)] = jnp.concatenate(px + pm + [zeros8] * (pad // 8), axis=0).astype(BF16)

        def scores(g):
            n = groups[g][1]
            s = jax.lax.dot_general(stk.pop((0, g)), stk.pop((1, g)), NT, preferred_element_type=F32)
            s = s + bias_v[0 if n == 3 else 1, 0:nrows(n), :]
            m = jnp.max(s, axis=-1, keepdims=True)
            p = jnp.exp2((s - m) * c_exp)
            l = jnp.sum(p, axis=-1, keepdims=True)
            r = pl.reciprocal(l, approx=True)
            r = r * (2.0 - l * r)
            pr[g] = (p * r).astype(BF16)

        def pv(g):
            g0, n = groups[g]
            o3 = jnp.dot(pr.pop(g), stk.pop((2, g)), preferred_element_type=F32)
            for i in range(n):
                hh = g0 + i
                ox = o3[i * SEG:(i + 1) * SEG]
                om = o3[n * SEG + i * NM:n * SEG + (i + 1) * NM]
                if even:
                    o_v[hh, 0:32, :] = jnp.concatenate([ox[0:24], om], axis=0).astype(BF16)
                    stash_o[hh] = ox[24:32]
                else:
                    o_v[hh] = jnp.concatenate([stash_o[hh], om, ox], axis=0).astype(BF16)

        MO = 32 if even else 48

        def oproj(ga, gb, acc=None):
            h0_ = groups[ga][0]
            h1_ = groups[gb - 1][0] + groups[gb - 1][1]
            cols = []
            for n in range(D // 128):
                lhs = jnp.concatenate(
                    [pltpu.bitcast(o_u[hh, 0:MO // 2, :], BF16) for hh in range(h0_, h1_)], axis=1)
                w = pltpu.bitcast(wo_u[n, h0_ * E // 2:h1_ * E // 2, :], BF16)
                y = jnp.dot(lhs, w, preferred_element_type=F32)
                cols.append(y if acc is None else y + acc[n])
            return cols

        for g in range(NG):
            run_fill(g)
            proj(1, g)
            if even and g - pv_delay >= 0:
                pv(g - pv_delay)
            proj(0, g)
            if not even and g - pv_delay >= 0:
                proj(2, g, functools.partial(pv, g - pv_delay), 3 if groups[g][1] == 3 else 0)
            else:
                proj(2, g)
            scores(g)
        rest = list(range(NG - pv_delay, NG))
        res = oproj(0, 3)
        for g in rest[:-1]:
            pv(g)
        res = oproj(3, 7, res)
        pv(rest[-1])
        res = oproj(7, NG - 1, res)
        res = oproj(NG - 1, NG, res)
        run_fill('end')
        return jnp.concatenate(res, axis=1)

    def convert(r0, n=64):
        gt = jnp.concatenate([gate_v[pl.ds(r0, n), :]] * (D // 128), axis=1)
        o = gt * acc_a[pl.ds(r0, n), :] + acc_b[pl.ds(r0, n), :]
        out_v[pl.ds(r0, n), :] = o.astype(BF16)

    def out_copy(r0):
        return pltpu.make_async_copy(rows(out_v, r0, 64), rows(out_hbm, r0, 64), sems.at[OUT_SEM])

    def super_step(r0, mem, fills):
        xa = x_v[pl.ds(r0, 32), :]
        xmid = x_v[pl.ds(r0 + 32, 16), :].astype(F32)
        xb = x_v[pl.ds(r0 + 48, 16), :]
        h_e = jnp.concatenate(
            [xa, jnp.concatenate([xmid[:8], mem], axis=0).astype(BF16)], axis=0)
        res = sub_step(h_e, True, 2, fills[0])
        acc_a[pl.ds(r0, 24), :] = res[0:24]
        h_o = jnp.concatenate(
            [jnp.concatenate([res[24:32], xmid[8:]], axis=0).astype(BF16), xb], axis=0)
        res = sub_step(h_o, False, 2, fills[1])
        acc_a[pl.ds(r0 + 24, 8), :] = res[0:8]
        acc_a[pl.ds(r0 + 32, 32), :] = res[16:48]
        return res[8:16]

    def body(i, carry):
        r0 = pl.multiple_of(i * (64 * UNROLL), 64 * UNROLL)
        fr = pl.multiple_of(F0 + (i // 2) * FR, FR)
        fo = pl.multiple_of((i % 2) * DFH, 128)

        def gu(c0, cw):
            def f():
                xf = x_v[pl.ds(fr, FR), :]
                if c0 == 0:
                    gate_v[pl.ds(fr, FR), :] = gate_of(xf)
                omg = 1.0 - gate_v[pl.ds(fr, FR), :]
                g = jax.lax.dot_general(xf, wg_v[pl.ds(fo + c0, cw), :], NT, preferred_element_type=F32)
                u = jax.lax.dot_general(xf, wu_v[pl.ds(fo + c0, cw), :], NT, preferred_element_type=F32)
                hf_v[:, c0:c0 + cw] = act(g, u, omg)
            return f

        def down(c0, cw):
            def f():
                b = jnp.dot(hf_v[:, c0:c0 + cw], wd_v[pl.ds(fo + c0, cw), :], preferred_element_type=F32)
                acc_b[pl.ds(fr, FR), :] = acc_b[pl.ds(fr, FR), :] + b
            return f

        rp = pl.multiple_of(jnp.maximum(r0 - 64, 0), 64)

        def conv(base, q):
            return lambda: convert(base + 16 * q, 16)

        def emit():
            @pl.when(i > 0)
            def _():
                out_copy(rp).start()

            out_copy(r0).start()

        fills = [
            {1: [gu(0, 256)], 'end': [gu(256, 256)]},
            {4: [down(0, 256)], 'end': [gu(512, 256)]},
            {1: [conv(rp, 0)], 2: [down(256, 256), conv(rp, 1)], 3: [conv(rp, 2)], 4: [conv(rp, 3)],
             5: [gu(768, 128), conv(r0, 0)], 6: [conv(r0, 1)], 7: [conv(r0, 2)], 8: [conv(r0, 3)], 9: [emit],
             'end': [down(512, 384)]},
            {},
        ]
        mem = mem_v[...]
        for u in range(UNROLL):
            mem = super_step(r0 + 64 * u, mem, fills[2 * u:2 * u + 2])
        mem_v[...] = mem
        return carry

    jax.lax.fori_loop(0, NBODY, body, 0)

    convert(S - 64)
    out_copy(S - 64).start()
    pltpu.make_async_copy(out_v, out_hbm, sems.at[OUT_SEM]).wait()


@functools.partial(jax.jit, static_argnames=("A_seg_len",))
def pallas_gated_mix__memory_aug_recurrent_mem_tr__glu_gated_geglu__prompt_kernel(
    A_x, A_mem0, A_Wq, A_Wk, A_Wv, A_Wo, A_seg_len, B_x, B_w_gate, B_w_up, B_w_down, gate_w,
):
    B, S, D = A_x.shape
    _, H, E = A_Wq.shape
    NM = A_mem0.shape[1]
    DF = B_w_gate.shape[1]
    SEG = int(A_seg_len)
    assert (B, S, D, H, E, NM, SEG, DF) == (1, 2048, 640, 32, 128, 8, 32, 1728)
    DFP = -(-DF // 256) * 256

    kernel = functools.partial(_kernel, S=S, D=D, H=H, E=E, NM=NM, SEG=SEG, DF=DF)
    hbm_spec = pl.BlockSpec(memory_space=pltpu.HBM)
    out = pl.pallas_call(
        kernel,
        out_shape=jax.ShapeDtypeStruct((S, D), BF16),
        in_specs=[hbm_spec] * 10,
        out_specs=hbm_spec,
        scratch_shapes=[
            pltpu.VMEM((S, D), BF16),
            pltpu.VMEM((NM, D), BF16),
            pltpu.VMEM((D,), BF16),
            pltpu.VMEM(((3 * D + DB) * H + 16, E), BF16),
            pltpu.VMEM((4 * H * 2 * WP, E), BF16),
            pltpu.VMEM((D // 128, H * E, 128), BF16),
            pltpu.VMEM((DFP, D), BF16),
            pltpu.VMEM((DFP, D), BF16),
            pltpu.VMEM((DFP, D), BF16),
            pltpu.VMEM((128, D), BF16),
            pltpu.VMEM((S, D), F32),
            pltpu.VMEM((S, D), F32),
            pltpu.VMEM((S, 128), F32),
            pltpu.VMEM((S, D), BF16),
            pltpu.VMEM((RB0, DF), BF16),
            pltpu.VMEM((FR, DFP // 2), BF16),
            pltpu.VMEM((NM, D), F32),
            pltpu.VMEM((3 * H, 8, E), F32),
            pltpu.VMEM((H, 8, E), F32),
            pltpu.VMEM((H, 48, E), BF16),
            pltpu.VMEM((2, 128, 128), F32),
            pltpu.SemaphoreType.DMA((35,)),
        ],
        compiler_params=pltpu.CompilerParams(vmem_limit_bytes=110 * 1024 * 1024),
    )(
        A_x.reshape(S, D), A_mem0.reshape(NM, D),
        A_Wq.reshape(D * H, E), A_Wk.reshape(D * H, E), A_Wv.reshape(D * H, E),
        A_Wo.reshape(H * E, D), B_w_gate.T, B_w_up.T, B_w_down, gate_w,
    )
    return out.reshape(B, S, D)
```
